```python
import jax
import jax.numpy as jnp

def _softmax(x, axis=-1):
    return jax.nn.softmax(x, axis=axis)
def _gelu(x):
    return jax.nn.gelu(x, approximate=True)
def _silu(x):
    return jax.nn.silu(x)
def _sigmoid(x):
    return jax.nn.sigmoid(x)
def _layernorm(x, axis=-1, eps=1e-5):
    m = jnp.mean(x, axis=axis, keepdims=True)
    v = jnp.var(x, axis=axis, keepdims=True)
    return (x - m) / jnp.sqrt(v + eps)
def _scatter_add(tgt, idx, src, axis=0):
    return tgt.at[idx].add(src)
def _segment_sum(src, seg, n):
    return jax.ops.segment_sum(src, seg, n)
class _Rng:
    def __init__(self, key):
        self._k = key
    def _next(self):
        self._k, sub = jax.random.split(self._k)
        return sub
    def normal(self, shape):
        return jax.random.normal(self._next(), shape, dtype=jnp.bfloat16)
    def randint(self, lo, hi, shape):
        return jax.random.randint(self._next(), shape, lo, hi, dtype=jnp.int32)
    def uniform(self, shape, lo=0.0, hi=1.0):
        return jax.random.uniform(self._next(), shape, jnp.bfloat16, lo, hi)
    def permutation(self, n):
        return jax.random.permutation(self._next(), n)


kernel_name = 'parallel_sum__ssm_conv_s5__moe_arch_mod__prompt'

def setup_inputs():
    _rng = _Rng(jax.random.key(int.from_bytes(__import__("os").urandom(4), "little")))
    _w = (lambda a: (lambda t: t.astype(jnp.bfloat16) if jnp.issubdtype(t.dtype, jnp.floating) else t)(jnp.asarray(a)))
    def _A_setup():
        B, S, D = 1, 2048, 1024
        P = D
        Lambda_re = -0.5 * jnp.exp((lambda *s: _rng.normal(s) * 0.05)(P))
        Lambda_im = (lambda *s: _rng.normal(s) * 0.05)(P) * 1.0
        B_re = (lambda *s: _rng.normal(s) * 0.05)(P, D) * (D ** -0.5)
        B_im = (lambda *s: _rng.normal(s) * 0.05)(P, D) * (D ** -0.5)
        C_re = (lambda *s: _rng.normal(s) * 0.05)(D, P) * (P ** -0.5)
        C_im = (lambda *s: _rng.normal(s) * 0.05)(D, P) * (P ** -0.5)
        log_dt = (lambda *s: _rng.normal(s) * 0.05)(P) * 0.3 - 2.0
        Dskip = (lambda *s: _rng.normal(s) * 0.05)(D)
        return {
            "x": _w((lambda *s: _rng.normal(s) * 0.05)(B, S, D)),
            "Lambda_re": _w(Lambda_re),
            "Lambda_im": _w(Lambda_im),
            "B_re": _w(B_re),
            "B_im": _w(B_im),
            "C_re": _w(C_re),
            "C_im": _w(C_im),
            "log_dt": _w(log_dt),
            "Dskip": _w(Dskip),
        }
    _A_in = _A_setup()

    def _B_setup():
        B, S, D, F, C = 1, 2048, 1024, 3584, 2
        return {
            "x": _w((lambda *s: _rng.normal(s) * 0.05)(B, S, D)),
            "w_r": _w((lambda *s: _rng.normal(s) * 0.05)(D)),
            "w_gate": _w((lambda *s: _rng.normal(s) * 0.05)(D, F)),
            "w_up": _w((lambda *s: _rng.normal(s) * 0.05)(D, F)),
            "w_down": _w((lambda *s: _rng.normal(s) * 0.05)(F, D)),
        }
    _B_in = _B_setup()

    return {
        "A_x": _A_in["x"],
        "A_Lambda_re": _A_in["Lambda_re"],
        "A_Lambda_im": _A_in["Lambda_im"],
        "A_B_re": _A_in["B_re"],
        "A_B_im": _A_in["B_im"],
        "A_C_re": _A_in["C_re"],
        "A_C_im": _A_in["C_im"],
        "A_log_dt": _A_in["log_dt"],
        "A_Dskip": _A_in["Dskip"],
        "B_x": _B_in["x"],
        "B_w_r": _B_in["w_r"],
        "B_w_gate": _B_in["w_gate"],
        "B_w_up": _B_in["w_up"],
        "B_w_down": _B_in["w_down"],
    }

def reference(A_x, A_Lambda_re, A_Lambda_im, A_B_re, A_B_im, A_C_re, A_C_im, A_log_dt, A_Dskip, B_x, B_w_r, B_w_gate, B_w_up, B_w_down):
    def _A_ref(x, Lambda_re, Lambda_im, B_re, B_im, C_re, C_im, log_dt, Dskip):
        Bsz, L, H = x.shape
        Lam = Lambda_re + 1j * Lambda_im
        Bmat = B_re + 1j * B_im
        Cmat = C_re + 1j * C_im
        dt = jnp.exp(log_dt)
        Lam_bar = jnp.exp(dt * Lam)
        B_bar = ((Lam_bar - 1.0) / Lam)[:, None] * Bmat
        Bu = jnp.einsum("bld,pd->blp", x + 0j, B_bar)
        h = jnp.zeros_like(Bu[:, 0, :])
        hs = []
        for t in range(L):
            h = Lam_bar[None, :] * h + Bu[:, t, :]
            hs.append(h)
        hseq = jnp.stack(hs, 1)
        y = 2.0 * jnp.einsum("blp,dp->bld", hseq, Cmat).real + x * Dskip[None, None, :]
        return y

    def _B_ref(x, w_r, w_gate, w_up, w_down):
        B, S, D = x.shape
        C = 2
        r = x @ w_r
        idx = jnp.argsort(-r, axis=-1)[:, :C]
        idx_e = jnp.repeat(idx.reshape(B, C, 1), D, axis=2)
        x_sel = jnp.take_along_axis(x, idx_e, axis=1)
        g = _silu(x_sel @ w_gate)
        u = x_sel @ w_up
        y = (g * u) @ w_down
        r_sel = _sigmoid(jnp.take_along_axis(r, idx, axis=1))
        y = y * r_sel.reshape(B, C, 1)
        b_off = (jnp.arange(B) * S).reshape(B, 1)
        flat_idx = (idx + b_off).reshape(B * C)
        zero = (x * 0.0).reshape(B * S, D)
        upd = _scatter_add(zero, flat_idx, y.reshape(B * C, D), axis=0)
        return x + upd.reshape(B, S, D)

    x = A_x
    xn = _layernorm(x, axis=-1)
    return x + _A_ref(xn, A_Lambda_re, A_Lambda_im, A_B_re, A_B_im, A_C_re, A_C_im, A_log_dt, A_Dskip) + _B_ref(xn, B_w_r, B_w_gate, B_w_up, B_w_down)
```

```python
import jax
import jax.numpy as jnp
from jax import lax
import jax.experimental.pallas as pl
import jax.experimental.pallas.tpu as pltpu

L, D, P, F = 2048, 1024, 1024, 3584
T = 256
NC = L // T
TP = T + 8
NT = P // 128
XW = 4
F32, BF16 = jnp.float32, jnp.bfloat16
_NT_DIMS = (((1,), (1,)), ((), ()))


def _rb(v):
    return v.astype(BF16).astype(F32)


def _discretize(lre, lim, ldt):
    lre, lim = lre.astype(F32), lim.astype(F32)
    dt = _rb(jnp.exp(ldt.astype(F32)))
    mag = jnp.exp(dt * lre)
    return lre, lim, mag * jnp.cos(dt * lim), mag * jnp.sin(dt * lim)


def _body(x_hbm, lre8, lim8, ldt8, lre1, lim1, ldt1, dsk, wr,
          bre_hbm, bim_hbm, cre_hbm, cim_hbm, wg_hbm, wu_hbm, wd_hbm,
          o_hbm,
          xv, bv, cv, cp, wg, wu, wd, buf, xnf, rs,
          ur0, ui0, ur1, ui1, hr0, hi0, hr1, hi1,
          sx, sw, so, sp):
    def xcopy(c):
        return pltpu.make_async_copy(x_hbm.at[pl.ds(c * T, T)], xv.at[pl.ds(c * T, T)], sx.at[c])

    def ocopy(c):
        return pltpu.make_async_copy(buf.at[pl.ds(c * T, T)], o_hbm.at[pl.ds(c * T, T)], so.at[c])

    wcopies = [pltpu.make_async_copy(s, d, sw.at[k]) for k, (s, d) in enumerate([
        (bre_hbm, bv.at[0]), (bim_hbm, bv.at[1]), (cre_hbm, cv.at[0]), (cim_hbm, cv.at[1]),
        (wg_hbm, wg), (wu_hbm, wu), (wd_hbm, wd)])]
    xcopy(0).start()
    wcopies[0].start()
    wcopies[1].start()
    xcopy(1).start()
    wcopies[2].start()
    wcopies[3].start()
    for c in range(2, NC):
        xcopy(c).start()
    for k in range(4, 7):
        wcopies[k].start()

    _, _, ar, ai = _discretize(lre8[...], lim8[...], ldt8[...])
    ubufs = ((ur0, ui0), (ur1, ui1))
    hbufs = ((hr0, hi0), (hr1, hi1))

    def stage_a(c, slot, first=False):
        xcopy(c).wait()
        rows = pl.ds(pl.multiple_of(c * T, T), T)
        x = xv[rows, :].astype(F32)
        mean = jnp.mean(x, axis=-1, keepdims=True)
        xc = x - mean
        var = _rb(jnp.mean(xc * xc, axis=-1, keepdims=True))
        den = _rb(jnp.sqrt(_rb(var + 1e-5)))
        xn = _rb(_rb(x - _rb(mean)) / den)
        xnf[rows, :] = xn
        rs[rows, :] = jnp.sum(xn * wr[...].astype(F32), axis=-1, keepdims=True)
        buf[rows, :] = x + xn + _rb(xn * dsk[...].astype(F32))
        xb = xn.astype(BF16)
        for k in range(2):
            if first:
                wcopies[k].wait()
            u = lax.dot_general(xb, bv[k], _NT_DIMS, preferred_element_type=F32)
            for s in range(NT):
                ubufs[slot][k][pl.ds(s * TP, T), :] = u[:, s * 128:(s + 1) * 128]

    def stage_s(slot, h):
        h_re, h_im = h
        (u_re, u_im), (o_re, o_im) = ubufs[slot], hbufs[slot]
        for t in range(T):
            idx = pl.ds(t, NT, stride=TP)
            n_re = (ar * h_re + u_re[idx, :]) - ai * h_im
            n_im = (ar * h_im + u_im[idx, :]) + ai * h_re
            h_re, h_im = n_re, n_im
            o_re[idx, :] = h_re
            o_im[idx, :] = h_im
        return h_re, h_im

    def stage_c(c, slot):
        rows = pl.ds(pl.multiple_of(c * T, T), T)
        y = buf[rows, :]
        for k in range(2):
            hb = jnp.concatenate(
                [hbufs[slot][k][pl.ds(s * TP, T), :].astype(BF16) for s in range(NT)], axis=1)
            y = y + lax.dot_general(hb, cp[k], _NT_DIMS, preferred_element_type=F32)
        buf[rows, :] = y
        ocopy(c).start()

    def prep_c():
        lre, lim, br, bi = _discretize(lre1[...], lim1[...], ldt1[...])
        br = br - 1.0
        inv = 2.0 / (lre * lre + lim * lim)
        cr = (br * lre + bi * lim) * inv
        ci = (bi * lre - br * lim) * inv
        wcopies[2].wait()
        wcopies[3].wait()
        c_re, c_im = cv[0].astype(F32), cv[1].astype(F32)
        cp[0] = (c_re * cr - c_im * ci).astype(BF16)
        cp[1] = (-(c_re * ci + c_im * cr)).astype(BF16)

    def ffn():
        r = _rb(rs[...])
        row = lax.broadcasted_iota(jnp.int32, r.shape, 0)
        m1 = jnp.max(r)
        i1 = jnp.min(jnp.where(r == m1, row, L))
        r2 = jnp.where(row == i1, -jnp.inf, r)
        m2 = jnp.max(r2)
        i2 = jnp.min(jnp.where(r2 == m2, row, L))
        i1 = jnp.clip(i1, 0, L - 1)
        i2 = jnp.clip(i2, 0, L - 1)
        sub = lax.broadcasted_iota(jnp.int32, (16, D), 0)
        xs = jnp.where(sub == 0, xnf[pl.ds(i1, 1), :], jnp.where(sub == 1, xnf[pl.ds(i2, 1), :], 0.0))
        xs = xs.astype(BF16)
        for k in range(4, 7):
            wcopies[k].wait()
        g = _rb(jnp.dot(xs, wg[...], preferred_element_type=F32))
        u = _rb(jnp.dot(xs, wu[...], preferred_element_type=F32))
        a = (_rb(g * jax.nn.sigmoid(g)) * u).astype(BF16)
        y = _rb(jnp.dot(a, wd[...], preferred_element_type=F32))
        sub1 = lax.broadcasted_iota(jnp.int32, (16, 1), 0)
        gate = _rb(jax.nn.sigmoid(jnp.where(sub1 == 0, m1, m2)))
        y = _rb(y * gate)
        return i1, i2, y

    zero = jnp.zeros((NT, 128), F32)
    stage_a(0, 0, first=True)
    prep_c()
    stage_a(1, 1)
    h = stage_s(0, (zero, zero))

    def loop(j, h):
        c = 2 * j + 2
        stage_a(c, 0)
        h = stage_s(1, h)
        stage_c(c - 2, 0)
        stage_a(c + 1, 1)
        h = stage_s(0, h)
        stage_c(c - 1, 1)
        return h

    h = lax.fori_loop(0, (NC - 2) // 2, loop, h)

    i1, i2, y = ffn()
    stage_s(1, h)
    for c in range(NC - 2):
        ocopy(c).wait()
    buf[pl.ds(i1, 1), :] = buf[pl.ds(i1, 1), :] + y[0:1]
    buf[pl.ds(i2, 1), :] = buf[pl.ds(i2, 1), :] + y[1:2]

    def pcopy(i, k):
        g = pl.ds(pl.multiple_of((i // 8) * 8, 8), 8)
        return pltpu.make_async_copy(buf.at[g], o_hbm.at[g], sp.at[k])

    done = (NC - 2) * T
    p1 = i1 < done
    p2 = jnp.logical_and(i2 < done, i2 // 8 != i1 // 8)
    pl.when(p1)(lambda: pcopy(i1, 0).start())
    pl.when(p2)(lambda: pcopy(i2, 1).start())
    stage_c(NC - 2, 0)
    stage_c(NC - 1, 1)
    pl.when(p1)(lambda: pcopy(i1, 0).wait())
    pl.when(p2)(lambda: pcopy(i2, 1).wait())
    ocopy(NC - 2).wait()
    ocopy(NC - 1).wait()


@jax.jit
def pallas_parallel_sum__ssm_conv_s5__moe_arch_mod__prompt_kernel(
    A_x, A_Lambda_re, A_Lambda_im, A_B_re, A_B_im, A_C_re, A_C_im, A_log_dt, A_Dskip,
    B_x, B_w_r, B_w_gate, B_w_up, B_w_down,
):
    del B_x
    hbm = pl.BlockSpec(memory_space=pl.ANY)
    vm = pl.BlockSpec(memory_space=pltpu.VMEM)
    scan_buf = pltpu.VMEM((NT * TP, 128), F32)
    out = pl.pallas_call(
        _body,
        out_shape=jax.ShapeDtypeStruct((L, D), F32),
        in_specs=[hbm] + [vm] * 8 + [hbm] * 7,
        out_specs=hbm,
        scratch_shapes=[
            pltpu.VMEM((L, D), BF16), pltpu.VMEM((2, P, D), BF16), pltpu.VMEM((2, D, P), BF16),
            pltpu.VMEM((2, D, P), BF16),
            pltpu.VMEM((D, F), BF16), pltpu.VMEM((D, F), BF16), pltpu.VMEM((F, D), BF16),
            pltpu.VMEM((L, D), F32), pltpu.VMEM((L, D), F32), pltpu.VMEM((L, 1), F32),
        ] + [scan_buf] * 8 + [
            pltpu.SemaphoreType.DMA((NC,)), pltpu.SemaphoreType.DMA((7,)),
            pltpu.SemaphoreType.DMA((NC,)), pltpu.SemaphoreType.DMA((2,)),
        ],
        compiler_params=pltpu.CompilerParams(vmem_limit_bytes=100 * 1024 * 1024),
    )(
        A_x.reshape(L, D),
        A_Lambda_re.reshape(NT, 128), A_Lambda_im.reshape(NT, 128), A_log_dt.reshape(NT, 128),
        A_Lambda_re.reshape(1, P), A_Lambda_im.reshape(1, P), A_log_dt.reshape(1, P),
        A_Dskip.reshape(1, D), B_w_r.reshape(1, D),
        A_B_re, A_B_im, A_C_re, A_C_im, B_w_gate, B_w_up, B_w_down,
    )
    return out.reshape(1, L, D)
```

```python
import jax
import jax.numpy as jnp
from jax import lax
import jax.experimental.pallas as pl
import jax.experimental.pallas.tpu as pltpu

L, D, P, F = 2048, 1024, 1024, 3584
T = 256
NC = L // T
TP = T + 8
NT = P // 128
TS = 4
F32, BF16 = jnp.float32, jnp.bfloat16
_NT_DIMS = (((1,), (1,)), ((), ()))


def _rb(v):
    return v.astype(BF16).astype(F32)


def _after(v, tok):
    return v


def _discretize(lre, lim, ldt):
    lre, lim = lre.astype(F32), lim.astype(F32)
    dt = _rb(jnp.exp(ldt.astype(F32)))
    mag = jnp.exp(dt * lre)
    return lre, lim, mag * jnp.cos(dt * lim), mag * jnp.sin(dt * lim)


def _body(x_hbm, lre8, lim8, ldt8, lre1, lim1, ldt1, dsk, wr,
          bre_hbm, bim_hbm, cre_hbm, cim_hbm, wg_hbm, wu_hbm, wd_hbm,
          o_hbm,
          xv, bv, cv, cp, wg, wu, wd, buf, xnf, xnb, rs,
          ur0, ui0, ur1, ui1, hr0, hi0, hr1, hi1,
          sx, sw, so, sp, st):
    def xcopy(c):
        return pltpu.make_async_copy(x_hbm.at[pl.ds(c * T, T)], xv.at[pl.ds(c * T, T)], sx.at[c])

    def ocopy(c):
        return pltpu.make_async_copy(buf.at[pl.ds(c * T, T)], o_hbm.at[pl.ds(c * T, T)], so.at[c])

    wcopies = [pltpu.make_async_copy(s, d, sw.at[k]) for k, (s, d) in enumerate([
        (bre_hbm, bv.at[0]), (bim_hbm, bv.at[1]), (cre_hbm, cv.at[0]), (cim_hbm, cv.at[1]),
        (wg_hbm, wg), (wu_hbm, wu), (wd_hbm, wd)])]
    xcopy(0).start()
    wcopies[0].start()
    wcopies[1].start()
    xcopy(1).start()
    wcopies[2].start()
    wcopies[3].start()
    for c in range(2, NC):
        xcopy(c).start()

    _, _, ar, ai = _discretize(lre8[...], lim8[...], ldt8[...])
    ubufs = ((ur0, ui0), (ur1, ui1))
    hbufs = ((hr0, hi0), (hr1, hi1))

    def stage_ln(c, q):
        rows, rr = pl.ds(c * T + q * 32, 32), pl.ds(q * 32, 32)
        x = xv[rows, :].astype(F32)
        mean = jnp.mean(x, axis=-1, keepdims=True)
        xc = x - mean
        var = _rb(jnp.mean(xc * xc, axis=-1, keepdims=True))
        den = _rb(jnp.sqrt(_rb(var + 1e-5)))
        xn = _rb(_rb(x - _rb(mean)) / den)
        xnf[rows, :] = xn
        r = jnp.sum(xn * wr[...].astype(F32), axis=-1, keepdims=True)
        lane = lax.broadcasted_iota(jnp.int32, (32, 128), 1)
        rs[rr, :] = jnp.where(lane == c, r, rs[rr, :] if c else -jnp.inf)
        buf[rows, :] = x + xn + _rb(xn * dsk[...].astype(F32))
        xnb[rows, :] = xn.astype(BF16)
        return r

    def stage_a(c, first=False, mid=None):
        slot = c % 2
        xb = xnb[pl.ds(c * T, T), :]
        for k in range(2):
            for n in range(4):
                u = lax.dot_general(xb, bv[k, pl.ds(n * 256, 256), :], _NT_DIMS,
                                    preferred_element_type=F32)
                for s in range(2):
                    ubufs[slot][k][pl.ds((2 * n + s) * TP, T), :] = u[:, s * 128:(s + 1) * 128]
                if mid is not None:
                    tok = mid(4 * k + n)
                    xb = _after(xb, tok)

    def stage_s(slot, h):
        h_re, h_im = h
        (u_re, u_im), (o_re, o_im) = ubufs[slot], hbufs[slot]
        for t in range(T):
            idx = pl.ds(t, NT, stride=TP)
            n_re = (ar * h_re + u_re[idx, :]) - ai * h_im
            n_im = (ar * h_im + u_im[idx, :]) + ai * h_re
            h_re, h_im = n_re, n_im
            o_re[idx, :] = h_re
            o_im[idx, :] = h_im
        return h_re, h_im

    def stage_c(c, cols=pl.ds(0, D), tok=None):
        slot = c % 2
        rows = pl.ds(c * T, T)
        y = buf[rows, cols]
        for k in range(2):
            hb = jnp.concatenate(
                [hbufs[slot][k][pl.ds(s * TP, T), :].astype(BF16) for s in range(NT)], axis=1)
            if tok is not None and k == 1:
                hb = _after(hb, tok)
            y = y + lax.dot_general(hb, cp[k, cols, :], _NT_DIMS, preferred_element_type=F32)
        buf[rows, cols] = y

    def coef():
        lre, lim, br, bi = _discretize(lre1[...], lim1[...], ldt1[...])
        br = br - 1.0
        inv = 2.0 / (lre * lre + lim * lim)
        cr = (br * lre + bi * lim) * inv
        ci = (bi * lre - br * lim) * inv
        return cr, ci

    def prep_c(q, cr, ci):
        for rows in [pl.ds(q * 128 + i, 16) for i in range(0, 128, 16)]:
            c_re, c_im = cv[0, rows].astype(F32), cv[1, rows].astype(F32)
            cp[0, rows] = (c_re * cr - c_im * ci).astype(BF16)
            cp[1, rows] = (c_im * -cr - c_re * ci).astype(BF16)

    def route():
        r = _rb(rs[...])
        row = (lax.broadcasted_iota(jnp.int32, r.shape, 0)
               + T * lax.broadcasted_iota(jnp.int32, r.shape, 1))
        m1 = jnp.max(r)
        i1 = jnp.min(jnp.where(r == m1, row, L))
        r2 = jnp.where(row == i1, -jnp.inf, r)
        m2 = jnp.max(r2)
        i2 = jnp.min(jnp.where(r2 == m2, row, L))
        i1 = jnp.clip(i1, 0, L - 1)
        i2 = jnp.clip(i2, 0, L - 1)
        sub = lax.broadcasted_iota(jnp.int32, (16, D), 0)
        xs = jnp.where(sub == 0, xnf[pl.ds(i1, 1), :], jnp.where(sub == 1, xnf[pl.ds(i2, 1), :], 0.0))
        return i1, i2, m1, m2, xs.astype(BF16)

    def ffn(m1, m2, xs):
        g = _rb(jnp.dot(xs, wg[...], preferred_element_type=F32))
        u = _rb(jnp.dot(xs, wu[...], preferred_element_type=F32))
        a = (_rb(g * jax.nn.sigmoid(g)) * u).astype(BF16)
        y = _rb(jnp.dot(a, wd[...], preferred_element_type=F32))
        sub1 = lax.broadcasted_iota(jnp.int32, (16, 1), 0)
        gate = _rb(jax.nn.sigmoid(jnp.where(sub1 == 0, m1, m2)))
        y = _rb(y * gate)
        return y

    zero = jnp.zeros((NT, 128), F32)
    xcopy(0).wait()
    for q in range(8):
        stage_ln(0, q)
    xcopy(1).wait()
    wcopies[0].wait()
    wcopies[1].wait()
    for k in range(4, 7):
        wcopies[k].start()
    stage_a(0, mid=lambda q: stage_ln(1, q))
    h = (zero, zero)
    for c in range(1, NC):
        if c + 1 < NC:
            xcopy(c + 1).wait()
        if c == 1:
            wcopies[2].wait()
            wcopies[3].wait()
        if c == 1:
            cr, ci = coef()
            stage_a(c, mid=lambda q: (prep_c(q, cr, ci), stage_ln(2, q))[1])
        elif c + 1 < NC:
            stage_a(c, mid=lambda q: stage_ln(c + 1, q))
        else:
            stage_a(c)
            i1, i2, m1, m2, xs = route()
        h = stage_s((c - 1) % 2, h)
        if c >= 2:
            stage_c(c - 2, tok=h[0])
        if c >= 2:
            ocopy(c - 2).start()
    for k in range(4, 7):
        wcopies[k].wait()
    y = ffn(m1, m2, xs)
    h = stage_s(1, h)
    stage_c(NC - 2, tok=h[0])
    for c in range(NC - 2):
        ocopy(c).wait()
    buf[pl.ds(i1, 1), :] = buf[pl.ds(i1, 1), :] + y[0:1]
    buf[pl.ds(i2, 1), :] = buf[pl.ds(i2, 1), :] + y[1:2]

    def pcopy(i, k):
        g = pl.ds(pl.multiple_of((i // 8) * 8, 8), 8)
        return pltpu.make_async_copy(buf.at[g], o_hbm.at[g], sp.at[k])

    done = (NC - 2) * T
    p1 = i1 < done
    p2 = jnp.logical_and(i2 < done, i2 // 8 != i1 // 8)
    pl.when(p1)(lambda: pcopy(i1, 0).start())
    pl.when(p2)(lambda: pcopy(i2, 1).start())
    ocopy(NC - 2).start()
    tails = []
    for q in range(TS):
        cols = pl.ds(q * (D // TS), D // TS)
        stage_c(NC - 1, cols)
        rows = pl.ds(L - T, T)
        tails.append(pltpu.make_async_copy(buf.at[rows, cols], o_hbm.at[rows, cols], st.at[q]))
        tails[-1].start()
    pl.when(p1)(lambda: pcopy(i1, 0).wait())
    pl.when(p2)(lambda: pcopy(i2, 1).wait())
    ocopy(NC - 2).wait()
    for t in tails:
        t.wait()


@jax.jit
def pallas_parallel_sum__ssm_conv_s5__moe_arch_mod__prompt_kernel(
    A_x, A_Lambda_re, A_Lambda_im, A_B_re, A_B_im, A_C_re, A_C_im, A_log_dt, A_Dskip,
    B_x, B_w_r, B_w_gate, B_w_up, B_w_down,
):
    del B_x
    hbm = pl.BlockSpec(memory_space=pl.ANY)
    vm = pl.BlockSpec(memory_space=pltpu.VMEM)
    scan_buf = pltpu.VMEM((NT * TP, 128), F32)
    out = pl.pallas_call(
        _body,
        out_shape=jax.ShapeDtypeStruct((L, D), F32),
        in_specs=[hbm] + [vm] * 8 + [hbm] * 7,
        out_specs=hbm,
        scratch_shapes=[
            pltpu.VMEM((L, D), BF16), pltpu.VMEM((2, P, D), BF16), pltpu.VMEM((2, D, P), BF16),
            pltpu.VMEM((2, D, P), BF16),
            pltpu.VMEM((D, F), BF16), pltpu.VMEM((D, F), BF16), pltpu.VMEM((F, D), BF16),
            pltpu.VMEM((L, D), F32), pltpu.VMEM((L, D), F32), pltpu.VMEM((L, D), BF16), pltpu.VMEM((T, 128), F32),
        ] + [scan_buf] * 8 + [
            pltpu.SemaphoreType.DMA((NC,)), pltpu.SemaphoreType.DMA((7,)),
            pltpu.SemaphoreType.DMA((NC,)), pltpu.SemaphoreType.DMA((2,)),
            pltpu.SemaphoreType.DMA((TS,)),
        ],
        compiler_params=pltpu.CompilerParams(flags={'XLA_TPU_EVENLY_DISTRIBUTE_CRITICAL_NODES': True},
            vmem_limit_bytes=100 * 1024 * 1024),
    )(
        A_x.reshape(L, D),
        A_Lambda_re.reshape(NT, 128), A_Lambda_im.reshape(NT, 128), A_log_dt.reshape(NT, 128),
        A_Lambda_re.reshape(1, P), A_Lambda_im.reshape(1, P), A_log_dt.reshape(1, P),
        A_Dskip.reshape(1, D), B_w_r.reshape(1, D),
        A_B_re, A_B_im, A_C_re, A_C_im, B_w_gate, B_w_up, B_w_down,
    )
    return out.reshape(1, L, D)
```

```python
import jax
import jax.numpy as jnp
from jax import lax
import jax.experimental.pallas as pl
import jax.experimental.pallas.tpu as pltpu

L, D, P, F = 2048, 1024, 1024, 3584
T = 256
NC = L // T
TP = T + 8
NT = P // 128
TS = 4
AHEAD = 2
F32, BF16 = jnp.float32, jnp.bfloat16
_NT_DIMS = (((1,), (1,)), ((), ()))


def _rb(v):
    return v.astype(BF16).astype(F32)


def _discretize(lre, lim, ldt):
    lre, lim = lre.astype(F32), lim.astype(F32)
    dt = _rb(jnp.exp(ldt.astype(F32)))
    mag = jnp.exp(dt * lre)
    return lre, lim, mag * jnp.cos(dt * lim), mag * jnp.sin(dt * lim)


def _body(x_hbm, lre8, lim8, ldt8, lre1, lim1, ldt1, dsk, wr,
          bre_hbm, bim_hbm, cre_hbm, cim_hbm, wg_hbm, wu_hbm, wd_hbm,
          o_hbm,
          xv, bv, cv, cp, wg, wu, wd, buf, xnf, xnb, rs,
          ur0, ui0, ur1, ui1, hr0, hi0, hr1, hi1,
          sx, sw, so, sp, st, sb):
    def xcopy(c):
        return pltpu.make_async_copy(x_hbm.at[pl.ds(c * T, T)], xv.at[pl.ds(c * T, T)], sx.at[c])

    def ocopy(c):
        return pltpu.make_async_copy(buf.at[pl.ds(c * T, T)], o_hbm.at[pl.ds(c * T, T)], so.at[c])

    wcopies = [pltpu.make_async_copy(s, d, sw.at[k]) for k, (s, d) in enumerate([
        (cre_hbm, cv.at[0]), (cim_hbm, cv.at[1]),
        (wg_hbm, wg), (wu_hbm, wu), (wd_hbm, wd)])]
    def bcopy(j):
        rows = pl.ds((j % 4) * 256, 256)
        return pltpu.make_async_copy((bre_hbm, bim_hbm)[j // 4].at[rows], bv.at[j // 4, rows], sb.at[j])

    xcopy(0).start()
    for j in range(AHEAD):
        bcopy(j).start()

    _, _, ar, ai = _discretize(lre8[...], lim8[...], ldt8[...])
    ubufs = ((ur0, ui0), (ur1, ui1))
    hbufs = ((hr0, hi0), (hr1, hi1))

    def stage_ln(c, q):
        rows, rr = pl.ds(c * T + q * 32, 32), pl.ds(q * 32, 32)
        x = xv[rows, :].astype(F32)
        mean = jnp.mean(x, axis=-1, keepdims=True)
        xc = x - mean
        var = _rb(jnp.mean(xc * xc, axis=-1, keepdims=True))
        den = _rb(jnp.sqrt(_rb(var + 1e-5)))
        xn = _rb(_rb(x - _rb(mean)) / den)
        xnf[rows, :] = xn
        r = jnp.sum(xn * wr[...].astype(F32), axis=-1, keepdims=True)
        lane = lax.broadcasted_iota(jnp.int32, (32, 128), 1)
        rs[rr, :] = jnp.where(lane == c, r, rs[rr, :] if c else -jnp.inf)
        buf[rows, :] = x + xn + _rb(xn * dsk[...].astype(F32))
        xnb[rows, :] = xn.astype(BF16)

    def stage_a(c, pre=None, mid=None):
        slot = c % 2
        xb = xnb[pl.ds(c * T, T), :]
        for k in range(2):
            for n in range(4):
                if pre is not None:
                    pre(4 * k + n)
                u = lax.dot_general(xb, bv[k, pl.ds(n * 256, 256), :], _NT_DIMS,
                                    preferred_element_type=F32)
                for s in range(2):
                    ubufs[slot][k][pl.ds((2 * n + s) * TP, T), :] = u[:, s * 128:(s + 1) * 128]
                if mid is not None:
                    mid(4 * k + n)

    def stage_s(slot, h):
        h_re, h_im = h
        (u_re, u_im), (o_re, o_im) = ubufs[slot], hbufs[slot]
        for t in range(T):
            idx = pl.ds(t, NT, stride=TP)
            n_re = (ar * h_re + u_re[idx, :]) - ai * h_im
            n_im = (ar * h_im + u_im[idx, :]) + ai * h_re
            h_re, h_im = n_re, n_im
            o_re[idx, :] = h_re
            o_im[idx, :] = h_im
        return h_re, h_im

    def stage_c(c, cols=pl.ds(0, D)):
        slot = c % 2
        rows = pl.ds(c * T, T)
        y = buf[rows, cols]
        for k in range(2):
            hb = jnp.concatenate(
                [hbufs[slot][k][pl.ds(s * TP, T), :].astype(BF16) for s in range(NT)], axis=1)
            y = y + lax.dot_general(hb, cp[k, cols, :], _NT_DIMS, preferred_element_type=F32)
        buf[rows, cols] = y

    def coef():
        lre, lim, br, bi = _discretize(lre1[...], lim1[...], ldt1[...])
        br = br - 1.0
        inv = 2.0 / (lre * lre + lim * lim)
        cr = (br * lre + bi * lim) * inv
        ci = (bi * lre - br * lim) * inv
        return cr, ci

    def prep_c(q, cr, ci):
        for rows in [pl.ds(q * 128 + i, 16) for i in range(0, 128, 16)]:
            c_re, c_im = cv[0, rows].astype(F32), cv[1, rows].astype(F32)
            cp[0, rows] = (c_re * cr - c_im * ci).astype(BF16)
            cp[1, rows] = (c_im * -cr - c_re * ci).astype(BF16)

    def route():
        r = _rb(rs[...])
        row = (lax.broadcasted_iota(jnp.int32, r.shape, 0)
               + T * lax.broadcasted_iota(jnp.int32, r.shape, 1))
        m1 = jnp.max(r)
        i1 = jnp.min(jnp.where(r == m1, row, L))
        r2 = jnp.where(row == i1, -jnp.inf, r)
        m2 = jnp.max(r2)
        i2 = jnp.min(jnp.where(r2 == m2, row, L))
        i1 = jnp.clip(i1, 0, L - 1)
        i2 = jnp.clip(i2, 0, L - 1)
        sub = lax.broadcasted_iota(jnp.int32, (16, D), 0)
        xs = jnp.where(sub == 0, xnf[pl.ds(i1, 1), :], jnp.where(sub == 1, xnf[pl.ds(i2, 1), :], 0.0))
        return i1, i2, m1, m2, xs.astype(BF16)

    def ffn(m1, m2, xs):
        g = _rb(jnp.dot(xs, wg[...], preferred_element_type=F32))
        u = _rb(jnp.dot(xs, wu[...], preferred_element_type=F32))
        a = (_rb(g * jax.nn.sigmoid(g)) * u).astype(BF16)
        y = _rb(jnp.dot(a, wd[...], preferred_element_type=F32))
        sub1 = lax.broadcasted_iota(jnp.int32, (16, 1), 0)
        gate = _rb(jax.nn.sigmoid(jnp.where(sub1 == 0, m1, m2)))
        y = _rb(y * gate)
        return y

    zero = jnp.zeros((NT, 128), F32)
    xcopy(0).wait()
    for q in range(8):
        stage_ln(0, q)

    def pre0(j):
        bcopy(j).wait()
        if j + AHEAD < 8:
            bcopy(j + AHEAD).start()
        if j == 1:
            xcopy(1).start()
        if j == 4:
            xcopy(1).wait()
        if j == 8 - AHEAD:
            xcopy(2).start()
            wcopies[0].start()
            wcopies[1].start()

    def mid0(j):
        if j >= 4:
            stage_ln(1, 2 * j - 8)
            stage_ln(1, 2 * j - 7)

    stage_a(0, pre=pre0, mid=mid0)
    h = (zero, zero)
    for c in range(1, NC):
        if c == 1:
            xcopy(2).wait()
            xcopy(3).start()
        if c == 2:
            wcopies[0].wait()
            wcopies[1].wait()
            xcopy(3).wait()
            for cc in range(4, NC):
                xcopy(cc).start()
            for k in range(2, 5):
                wcopies[k].start()
        if 3 <= c < NC - 1:
            xcopy(c + 1).wait()
        if c == NC - 1:
            ocopy(0).wait()
        if c + 1 < NC:
            stage_a(c, mid=lambda q: stage_ln(c + 1, q))
        else:
            stage_a(c)
            i1, i2, m1, m2, xs = route()
        h = stage_s((c - 1) % 2, h)
        if c == 2:
            cr, ci = coef()
            for q in range(8):
                prep_c(q, cr, ci)
        if c >= 2:
            stage_c(c - 2)
        if c >= 2:
            ocopy(c - 2).start()
    for k in range(2, 5):
        wcopies[k].wait()
    y = ffn(m1, m2, xs)
    h = stage_s(1, h)
    stage_c(NC - 2)
    for c in range(1, NC - 2):
        ocopy(c).wait()
    buf[pl.ds(i1, 1), :] = buf[pl.ds(i1, 1), :] + y[0:1]
    buf[pl.ds(i2, 1), :] = buf[pl.ds(i2, 1), :] + y[1:2]

    def pcopy(i, k):
        g = pl.ds(pl.multiple_of((i // 8) * 8, 8), 8)
        return pltpu.make_async_copy(buf.at[g], o_hbm.at[g], sp.at[k])

    done = (NC - 2) * T
    p1 = i1 < done
    p2 = jnp.logical_and(i2 < done, i2 // 8 != i1 // 8)
    pl.when(p1)(lambda: pcopy(i1, 0).start())
    pl.when(p2)(lambda: pcopy(i2, 1).start())
    ocopy(NC - 2).start()
    tails = []
    for q in range(TS):
        cols = pl.ds(q * (D // TS), D // TS)
        stage_c(NC - 1, cols)
        rows = pl.ds(L - T, T)
        tails.append(pltpu.make_async_copy(buf.at[rows, cols], o_hbm.at[rows, cols], st.at[q]))
        tails[-1].start()
    pl.when(p1)(lambda: pcopy(i1, 0).wait())
    pl.when(p2)(lambda: pcopy(i2, 1).wait())
    ocopy(NC - 2).wait()
    for t in tails:
        t.wait()


@jax.jit
def pallas_parallel_sum__ssm_conv_s5__moe_arch_mod__prompt_kernel(
    A_x, A_Lambda_re, A_Lambda_im, A_B_re, A_B_im, A_C_re, A_C_im, A_log_dt, A_Dskip,
    B_x, B_w_r, B_w_gate, B_w_up, B_w_down,
):
    del B_x
    hbm = pl.BlockSpec(memory_space=pl.ANY)
    vm = pl.BlockSpec(memory_space=pltpu.VMEM)
    scan_buf = pltpu.VMEM((NT * TP, 128), F32)
    out = pl.pallas_call(
        _body,
        out_shape=jax.ShapeDtypeStruct((L, D), F32),
        in_specs=[hbm] + [vm] * 8 + [hbm] * 7,
        out_specs=hbm,
        scratch_shapes=[
            pltpu.VMEM((L, D), BF16), pltpu.VMEM((2, P, D), BF16), pltpu.VMEM((2, D, P), BF16),
            pltpu.VMEM((2, D, P), BF16),
            pltpu.VMEM((D, F), BF16), pltpu.VMEM((D, F), BF16), pltpu.VMEM((F, D), BF16),
            pltpu.VMEM((L, D), F32), pltpu.VMEM((L, D), F32), pltpu.VMEM((L, D), BF16), pltpu.VMEM((T, 128), F32),
        ] + [scan_buf] * 8 + [
            pltpu.SemaphoreType.DMA((NC,)), pltpu.SemaphoreType.DMA((5,)),
            pltpu.SemaphoreType.DMA((NC,)), pltpu.SemaphoreType.DMA((2,)),
            pltpu.SemaphoreType.DMA((TS,)), pltpu.SemaphoreType.DMA((8,)),
        ],
        compiler_params=pltpu.CompilerParams(flags={'XLA_TPU_EVENLY_DISTRIBUTE_CRITICAL_NODES': True},
            vmem_limit_bytes=100 * 1024 * 1024),
    )(
        A_x.reshape(L, D),
        A_Lambda_re.reshape(NT, 128), A_Lambda_im.reshape(NT, 128), A_log_dt.reshape(NT, 128),
        A_Lambda_re.reshape(1, P), A_Lambda_im.reshape(1, P), A_log_dt.reshape(1, P),
        A_Dskip.reshape(1, D), B_w_r.reshape(1, D),
        A_B_re, A_B_im, A_C_re, A_C_im, B_w_gate, B_w_up, B_w_down,
    )
    return out.reshape(1, L, D)
```

```python
import jax
import jax.numpy as jnp
from jax import lax
import jax.experimental.pallas as pl
import jax.experimental.pallas.tpu as pltpu

L, D, P, F = 2048, 1024, 1024, 3584
T = 256
NC = L // T
TP = T + 4
NT = P // 128
TS = 4
AHEAD = 3
F32, BF16 = jnp.float32, jnp.bfloat16
_NT_DIMS = (((1,), (1,)), ((), ()))


def _rb(v):
    return v.astype(BF16).astype(F32)


def _discretize(lre, lim, ldt):
    lre, lim = lre.astype(F32), lim.astype(F32)
    dt = _rb(jnp.exp(ldt.astype(F32)))
    mag = jnp.exp(dt * lre)
    return lre, lim, mag * jnp.cos(dt * lim), mag * jnp.sin(dt * lim)


def _body(x_hbm, lre8, lim8, ldt8, dsk, wr,
          bre_hbm, bim_hbm, cre_hbm, cim_hbm, wg_hbm, wu_hbm, wd_hbm,
          o_hbm,
          xv, bv, cv, wg, wu, wd, buf, xnf, xnb, rs,
          ur0, ui0, ur1, ui1, hr0, hi0, hr1, hi1,
          sx, sw, so, sp, st, sb):
    def xcopy(c):
        return pltpu.make_async_copy(x_hbm.at[pl.ds(c * T, T)], xv.at[pl.ds(c * T, T)], sx.at[c])

    def ocopy(c):
        return pltpu.make_async_copy(buf.at[pl.ds(c * T, T)], o_hbm.at[pl.ds(c * T, T)], so.at[c])

    wcopies = [pltpu.make_async_copy(s, d, sw.at[k]) for k, (s, d) in enumerate([
        (cre_hbm, cv.at[0]), (cim_hbm, cv.at[1]),
        (wg_hbm, wg), (wu_hbm, wu), (wd_hbm, wd)])]
    def bcopy(j):
        rows = pl.ds((j % 4) * 256, 256)
        return pltpu.make_async_copy((bre_hbm, bim_hbm)[j // 4].at[rows], bv.at[j // 4, rows], sb.at[j])

    xcopy(0).start()
    bcopy(0).start()

    _, _, ar, ai = _discretize(lre8[...], lim8[...], ldt8[...])
    ubufs = ((ur0, ui0), (ur1, ui1))
    hbufs = ((hr0, hi0), (hr1, hi1))

    def stage_ln(c, q):
        rows, rr = pl.ds(c * T + q * 32, 32), pl.ds(q * 32, 32)
        x = xv[rows, :].astype(F32)
        mean = jnp.mean(x, axis=-1, keepdims=True)
        xc = x - mean
        var = _rb(jnp.mean(xc * xc, axis=-1, keepdims=True))
        den = _rb(jnp.sqrt(_rb(var + 1e-5)))
        xn = _rb(_rb(x - _rb(mean)) / den)
        xnf[rows, :] = xn
        r = jnp.sum(xn * wr[...].astype(F32), axis=-1, keepdims=True)
        lane = lax.broadcasted_iota(jnp.int32, (32, 128), 1)
        rs[rr, :] = jnp.where(lane == c, r, rs[rr, :] if c else -jnp.inf)
        buf[rows, :] = x + xn + _rb(xn * dsk[...].astype(F32))
        xnb[rows, :] = xn.astype(BF16)

    def stage_a(c, pre=None, mid=None):
        slot = c % 2
        xb = xnb[pl.ds(c * T, T), :]
        for k in range(2):
            for n in range(4):
                if pre is not None:
                    pre(4 * k + n)
                u = lax.dot_general(xb, bv[k, pl.ds(n * 256, 256), :], _NT_DIMS,
                                    preferred_element_type=F32)
                for s in range(2):
                    ubufs[slot][k][pl.ds((2 * n + s) * TP, T), :] = u[:, s * 128:(s + 1) * 128]
                if mid is not None:
                    mid(4 * k + n)

    def stage_s(slot, h):
        h_re, h_im = h
        (u_re, u_im), (o_re, o_im) = ubufs[slot], hbufs[slot]
        for t in range(T):
            idx = pl.ds(t, NT, stride=TP)
            v_re, v_im = u_re[idx, :], u_im[idx, :]
            n_re = (ar * h_re + (cr * v_re - ci * v_im)) + ai * h_im
            n_im = (ar * h_im - (cr * v_im + ci * v_re)) - ai * h_re
            h_re, h_im = n_re, n_im
            o_re[idx, :] = h_re
            o_im[idx, :] = h_im
        return h_re, h_im

    def stage_c(c, cols=pl.ds(0, D)):
        slot = c % 2
        rows = pl.ds(c * T, T)
        y = buf[rows, cols]
        for k in range(2):
            hb = jnp.concatenate(
                [hbufs[slot][k][pl.ds(s * TP, T), :].astype(BF16) for s in range(NT)], axis=1)
            y = y + lax.dot_general(hb, cv[k, cols, :], _NT_DIMS, preferred_element_type=F32)
        buf[rows, cols] = y

    def coef():
        lre, lim, br, bi = _discretize(lre8[...], lim8[...], ldt8[...])
        br = br - 1.0
        inv = 2.0 / (lre * lre + lim * lim)
        cr = (br * lre + bi * lim) * inv
        ci = (bi * lre - br * lim) * inv
        return cr, ci

    def route():
        r = _rb(rs[...])
        row = (lax.broadcasted_iota(jnp.int32, r.shape, 0)
               + T * lax.broadcasted_iota(jnp.int32, r.shape, 1))
        m1 = jnp.max(r)
        i1 = jnp.min(jnp.where(r == m1, row, L))
        r2 = jnp.where(row == i1, -jnp.inf, r)
        m2 = jnp.max(r2)
        i2 = jnp.min(jnp.where(r2 == m2, row, L))
        i1 = jnp.clip(i1, 0, L - 1)
        i2 = jnp.clip(i2, 0, L - 1)
        sub = lax.broadcasted_iota(jnp.int32, (16, D), 0)
        xs = jnp.where(sub == 0, xnf[pl.ds(i1, 1), :], jnp.where(sub == 1, xnf[pl.ds(i2, 1), :], 0.0))
        return i1, i2, m1, m2, xs.astype(BF16)

    def ffn(m1, m2, xs):
        g = _rb(jnp.dot(xs, wg[...], preferred_element_type=F32))
        u = _rb(jnp.dot(xs, wu[...], preferred_element_type=F32))
        a = (_rb(g * jax.nn.sigmoid(g)) * u).astype(BF16)
        y = _rb(jnp.dot(a, wd[...], preferred_element_type=F32))
        sub1 = lax.broadcasted_iota(jnp.int32, (16, 1), 0)
        gate = _rb(jax.nn.sigmoid(jnp.where(sub1 == 0, m1, m2)))
        y = _rb(y * gate)
        return y

    cr, ci = coef()
    zero = jnp.zeros((NT, 128), F32)
    xcopy(0).wait()
    for j in range(1, AHEAD):
        bcopy(j).start()
    for q in range(8):
        stage_ln(0, q)

    def pre0(j):
        bcopy(j).wait()
        if j + AHEAD < 8:
            bcopy(j + AHEAD).start()
        if j == 1:
            xcopy(1).start()
        if j == 4:
            xcopy(1).wait()
        if j == 8 - AHEAD:
            xcopy(2).start()
            wcopies[0].start()
            wcopies[1].start()

    def mid0(j):
        if j >= 4:
            stage_ln(1, 2 * j - 8)
            stage_ln(1, 2 * j - 7)

    stage_a(0, pre=pre0, mid=mid0)
    h = (zero, zero)
    for c in range(1, NC):
        if c == 1:
            xcopy(2).wait()
            xcopy(3).start()
        if c == 2:
            wcopies[0].wait()
            wcopies[1].wait()
            xcopy(3).wait()
            for cc in range(4, NC):
                xcopy(cc).start()
            for k in range(2, 5):
                wcopies[k].start()
        if 3 <= c < NC - 1:
            xcopy(c + 1).wait()
        if c == NC - 1:
            ocopy(0).wait()
        if c + 1 < NC:
            stage_a(c, mid=lambda q: stage_ln(c + 1, q))
        else:
            stage_a(c)
            i1, i2, m1, m2, xs = route()
        h = stage_s((c - 1) % 2, h)
        if c >= 2:
            stage_c(c - 2)
        if c >= 2:
            ocopy(c - 2).start()
    for k in range(2, 5):
        wcopies[k].wait()
    y = ffn(m1, m2, xs)
    h = stage_s(1, h)
    stage_c(NC - 2)
    for c in range(1, NC - 2):
        ocopy(c).wait()
    buf[pl.ds(i1, 1), :] = buf[pl.ds(i1, 1), :] + y[0:1]
    buf[pl.ds(i2, 1), :] = buf[pl.ds(i2, 1), :] + y[1:2]

    def pcopy(i, k):
        g = pl.ds(pl.multiple_of((i // 8) * 8, 8), 8)
        return pltpu.make_async_copy(buf.at[g], o_hbm.at[g], sp.at[k])

    done = (NC - 2) * T
    p1 = i1 < done
    p2 = jnp.logical_and(i2 < done, i2 // 8 != i1 // 8)
    pl.when(p1)(lambda: pcopy(i1, 0).start())
    pl.when(p2)(lambda: pcopy(i2, 1).start())
    ocopy(NC - 2).start()
    tails = []
    for q in range(TS):
        cols = pl.ds(q * (D // TS), D // TS)
        stage_c(NC - 1, cols)
        rows = pl.ds(L - T, T)
        tails.append(pltpu.make_async_copy(buf.at[rows, cols], o_hbm.at[rows, cols], st.at[q]))
        tails[-1].start()
    pl.when(p1)(lambda: pcopy(i1, 0).wait())
    pl.when(p2)(lambda: pcopy(i2, 1).wait())
    ocopy(NC - 2).wait()
    for t in tails:
        t.wait()


@jax.jit
def pallas_parallel_sum__ssm_conv_s5__moe_arch_mod__prompt_kernel(
    A_x, A_Lambda_re, A_Lambda_im, A_B_re, A_B_im, A_C_re, A_C_im, A_log_dt, A_Dskip,
    B_x, B_w_r, B_w_gate, B_w_up, B_w_down,
):
    del B_x
    hbm = pl.BlockSpec(memory_space=pl.ANY)
    vm = pl.BlockSpec(memory_space=pltpu.VMEM)
    scan_buf = pltpu.VMEM((NT * TP, 128), F32)
    out = pl.pallas_call(
        _body,
        out_shape=jax.ShapeDtypeStruct((L, D), F32),
        in_specs=[hbm] + [vm] * 5 + [hbm] * 7,
        out_specs=hbm,
        scratch_shapes=[
            pltpu.VMEM((L, D), BF16), pltpu.VMEM((2, P, D), BF16), pltpu.VMEM((2, D, P), BF16),
            pltpu.VMEM((D, F), BF16), pltpu.VMEM((D, F), BF16), pltpu.VMEM((F, D), BF16),
            pltpu.VMEM((L, D), F32), pltpu.VMEM((L, D), F32), pltpu.VMEM((L, D), BF16), pltpu.VMEM((T, 128), F32),
        ] + [scan_buf] * 8 + [
            pltpu.SemaphoreType.DMA((NC,)), pltpu.SemaphoreType.DMA((5,)),
            pltpu.SemaphoreType.DMA((NC,)), pltpu.SemaphoreType.DMA((2,)),
            pltpu.SemaphoreType.DMA((TS,)), pltpu.SemaphoreType.DMA((8,)),
        ],
        compiler_params=pltpu.CompilerParams(flags={'XLA_TPU_EVENLY_DISTRIBUTE_CRITICAL_NODES': True},
            vmem_limit_bytes=100 * 1024 * 1024),
    )(
        A_x.reshape(L, D),
        A_Lambda_re.reshape(NT, 128), A_Lambda_im.reshape(NT, 128), A_log_dt.reshape(NT, 128),
        A_Dskip.reshape(1, D), B_w_r.reshape(1, D),
        A_B_re, A_B_im, A_C_re, A_C_im, B_w_gate, B_w_up, B_w_down,
    )
    return out.reshape(1, L, D)
```

```python
import jax
import jax.numpy as jnp
from jax import lax
import jax.experimental.pallas as pl
import jax.experimental.pallas.tpu as pltpu

L, D, P, F = 2048, 1024, 1024, 3584
T = 256
NC = L // T
TP = T + 4
NT = P // 128
TS = 4
AHEAD = 3
F32, BF16 = jnp.float32, jnp.bfloat16
_NT_DIMS = (((1,), (1,)), ((), ()))


def _rb(v):
    return v.astype(BF16).astype(F32)


def _discretize(lre, lim, ldt):
    lre, lim = lre.astype(F32), lim.astype(F32)
    dt = _rb(jnp.exp(ldt.astype(F32)))
    mag = jnp.exp(dt * lre)
    return lre, lim, mag * jnp.cos(dt * lim), mag * jnp.sin(dt * lim)


def _body(x_hbm, lre8, lim8, ldt8, lre1, lim1, ldt1, dsk, wr,
          bre_hbm, bim_hbm, cre_hbm, cim_hbm, wg_hbm, wu_hbm, wd_hbm,
          o_hbm,
          xv, bv, cv, cp, wg, wu, wd, buf, xnf, xnb, rs,
          ur0, ui0, ur1, ui1, hr0, hi0, hr1, hi1,
          sx, sw, so, sp, st, sb):
    def xcopy(c):
        return pltpu.make_async_copy(x_hbm.at[pl.ds(c * T, T)], xv.at[pl.ds(c * T, T)], sx.at[c])

    def ocopy(c):
        return pltpu.make_async_copy(buf.at[pl.ds(c * T, T)], o_hbm.at[pl.ds(c * T, T)], so.at[c])

    wcopies = [pltpu.make_async_copy(s, d, sw.at[k]) for k, (s, d) in enumerate([
        (cre_hbm, cv.at[0]), (cim_hbm, cv.at[1]),
        (wg_hbm, wg), (wu_hbm, wu), (wd_hbm, wd)])]
    def bcopy(j):
        rows = pl.ds((j % 4) * 256, 256)
        return pltpu.make_async_copy((bre_hbm, bim_hbm)[j // 4].at[rows], bv.at[j // 4, rows], sb.at[j])

    xcopy(0).start()
    bcopy(0).start()

    _, _, ar, ai = _discretize(lre8[...], lim8[...], ldt8[...])
    ubufs = ((ur0, ui0), (ur1, ui1))
    hbufs = ((hr0, hi0), (hr1, hi1))

    def stage_ln(c, q):
        rows, rr = pl.ds(c * T + q * 32, 32), pl.ds(q * 32, 32)
        x = xv[rows, :].astype(F32)
        mean = jnp.mean(x, axis=-1, keepdims=True)
        xc = x - mean
        var = _rb(jnp.mean(xc * xc, axis=-1, keepdims=True))
        den = _rb(jnp.sqrt(_rb(var + 1e-5)))
        xn = _rb(_rb(x - _rb(mean)) / den)
        xnf[rows, :] = xn
        r = jnp.sum(xn * wr[...].astype(F32), axis=-1, keepdims=True)
        lane = lax.broadcasted_iota(jnp.int32, (32, 128), 1)
        rs[rr, :] = jnp.where(lane == c, r, rs[rr, :] if c else -jnp.inf)
        buf[rows, :] = x + xn + _rb(xn * dsk[...].astype(F32))
        xnb[rows, :] = xn.astype(BF16)

    def stage_a(c, pre=None, mid=None):
        slot = c % 2
        xb = xnb[pl.ds(c * T, T), :]
        for k in range(2):
            for n in range(4):
                if pre is not None:
                    pre(4 * k + n)
                u = lax.dot_general(xb, bv[k, pl.ds(n * 256, 256), :], _NT_DIMS,
                                    preferred_element_type=F32)
                for s in range(2):
                    ubufs[slot][k][pl.ds((2 * n + s) * TP, T), :] = u[:, s * 128:(s + 1) * 128]
                if mid is not None:
                    mid(4 * k + n)

    def stage_s(slot, h):
        h_re, h_im = h
        (u_re, u_im), (o_re, o_im) = ubufs[slot], hbufs[slot]
        for t in range(T):
            idx = pl.ds(t, NT, stride=TP)
            n_re = (ar * h_re + u_re[idx, :]) - ai * h_im
            n_im = (ar * h_im + u_im[idx, :]) + ai * h_re
            h_re, h_im = n_re, n_im
            o_re[idx, :] = h_re
            o_im[idx, :] = h_im
        return h_re, h_im

    def stage_c(c, cols=pl.ds(0, D)):
        slot = c % 2
        rows = pl.ds(c * T, T)
        y = buf[rows, cols]
        for k in range(2):
            hb = jnp.concatenate(
                [hbufs[slot][k][pl.ds(s * TP, T), :].astype(BF16) for s in range(NT)], axis=1)
            y = y + lax.dot_general(hb, cp[k, cols, :], _NT_DIMS, preferred_element_type=F32)
        buf[rows, cols] = y

    def coef():
        lre, lim, br, bi = _discretize(lre1[...], lim1[...], ldt1[...])
        br = br - 1.0
        inv = 2.0 / (lre * lre + lim * lim)
        cr = (br * lre + bi * lim) * inv
        ci = (bi * lre - br * lim) * inv
        return cr, ci

    def prep_c(q, cr, ci):
        for rows in [pl.ds(q * 128 + i, 16) for i in range(0, 128, 16)]:
            c_re, c_im = cv[0, rows].astype(F32), cv[1, rows].astype(F32)
            cp[0, rows] = (c_re * cr - c_im * ci).astype(BF16)
            cp[1, rows] = (c_im * -cr - c_re * ci).astype(BF16)

    def route():
        r = _rb(rs[...])
        row = (lax.broadcasted_iota(jnp.int32, r.shape, 0)
               + T * lax.broadcasted_iota(jnp.int32, r.shape, 1))
        m1 = jnp.max(r)
        i1 = jnp.min(jnp.where(r == m1, row, L))
        r2 = jnp.where(row == i1, -jnp.inf, r)
        m2 = jnp.max(r2)
        i2 = jnp.min(jnp.where(r2 == m2, row, L))
        i1 = jnp.clip(i1, 0, L - 1)
        i2 = jnp.clip(i2, 0, L - 1)
        sub = lax.broadcasted_iota(jnp.int32, (16, D), 0)
        xs = jnp.where(sub == 0, xnf[pl.ds(i1, 1), :], jnp.where(sub == 1, xnf[pl.ds(i2, 1), :], 0.0))
        return i1, i2, m1, m2, xs.astype(BF16)

    def ffn(m1, m2, xs):
        g = _rb(jnp.dot(xs, wg[...], preferred_element_type=F32))
        u = _rb(jnp.dot(xs, wu[...], preferred_element_type=F32))
        a = (_rb(g * jax.nn.sigmoid(g)) * u).astype(BF16)
        y = _rb(jnp.dot(a, wd[...], preferred_element_type=F32))
        sub1 = lax.broadcasted_iota(jnp.int32, (16, 1), 0)
        gate = _rb(jax.nn.sigmoid(jnp.where(sub1 == 0, m1, m2)))
        y = _rb(y * gate)
        return y

    zero = jnp.zeros((NT, 128), F32)
    xcopy(0).wait()
    for j in range(1, AHEAD):
        bcopy(j).start()
    for q in range(8):
        stage_ln(0, q)

    def pre0(j):
        bcopy(j).wait()
        if j + AHEAD < 8:
            bcopy(j + AHEAD).start()
        if j == 1:
            xcopy(1).start()
        if j == 4:
            xcopy(1).wait()
        if j == 8 - AHEAD:
            xcopy(2).start()
            wcopies[0].start()
            wcopies[1].start()

    def mid0(j):
        if j >= 4:
            stage_ln(1, 2 * j - 8)
            stage_ln(1, 2 * j - 7)

    stage_a(0, pre=pre0, mid=mid0)
    h = (zero, zero)
    for c in range(1, NC):
        if c == 1:
            xcopy(2).wait()
            xcopy(3).start()
        if c == 2:
            wcopies[0].wait()
            wcopies[1].wait()
            xcopy(3).wait()
            for cc in range(4, NC):
                xcopy(cc).start()
            for k in range(2, 5):
                wcopies[k].start()
        if 3 <= c < NC - 1:
            xcopy(c + 1).wait()
        if c == NC - 1:
            ocopy(0).wait()
        if c + 1 < NC:
            stage_a(c, mid=lambda q: stage_ln(c + 1, q))
        else:
            stage_a(c)
            i1, i2, m1, m2, xs = route()
        h = stage_s((c - 1) % 2, h)
        if c == 2:
            cr, ci = coef()
            for q in range(4):
                prep_c(2 * q, cr, ci)
                prep_c(2 * q + 1, cr, ci)
                stage_c(0, pl.ds(q * 256, 256))
        if c > 2:
            stage_c(c - 2)
        if c >= 2:
            ocopy(c - 2).start()
    for k in range(2, 5):
        wcopies[k].wait()
    y = ffn(m1, m2, xs)
    h = stage_s(1, h)
    stage_c(NC - 2)
    for c in range(1, NC - 2):
        ocopy(c).wait()
    buf[pl.ds(i1, 1), :] = buf[pl.ds(i1, 1), :] + y[0:1]
    buf[pl.ds(i2, 1), :] = buf[pl.ds(i2, 1), :] + y[1:2]

    def pcopy(i, k):
        g = pl.ds(pl.multiple_of((i // 8) * 8, 8), 8)
        return pltpu.make_async_copy(buf.at[g], o_hbm.at[g], sp.at[k])

    done = (NC - 2) * T
    p1 = i1 < done
    p2 = jnp.logical_and(i2 < done, i2 // 8 != i1 // 8)
    pl.when(p1)(lambda: pcopy(i1, 0).start())
    pl.when(p2)(lambda: pcopy(i2, 1).start())
    ocopy(NC - 2).start()
    tails = []
    for q in range(TS):
        cols = pl.ds(q * (D // TS), D // TS)
        stage_c(NC - 1, cols)
        rows = pl.ds(L - T, T)
        tails.append(pltpu.make_async_copy(buf.at[rows, cols], o_hbm.at[rows, cols], st.at[q]))
        tails[-1].start()
    pl.when(p1)(lambda: pcopy(i1, 0).wait())
    pl.when(p2)(lambda: pcopy(i2, 1).wait())
    ocopy(NC - 2).wait()
    for t in tails:
        t.wait()


@jax.jit
def pallas_parallel_sum__ssm_conv_s5__moe_arch_mod__prompt_kernel(
    A_x, A_Lambda_re, A_Lambda_im, A_B_re, A_B_im, A_C_re, A_C_im, A_log_dt, A_Dskip,
    B_x, B_w_r, B_w_gate, B_w_up, B_w_down,
):
    del B_x
    hbm = pl.BlockSpec(memory_space=pl.ANY)
    vm = pl.BlockSpec(memory_space=pltpu.VMEM)
    scan_buf = pltpu.VMEM((NT * TP, 128), F32)
    out = pl.pallas_call(
        _body,
        out_shape=jax.ShapeDtypeStruct((L, D), F32),
        in_specs=[hbm] + [vm] * 8 + [hbm] * 7,
        out_specs=hbm,
        scratch_shapes=[
            pltpu.VMEM((L, D), BF16), pltpu.VMEM((2, P, D), BF16), pltpu.VMEM((2, D, P), BF16),
            pltpu.VMEM((2, D, P), BF16),
            pltpu.VMEM((D, F), BF16), pltpu.VMEM((D, F), BF16), pltpu.VMEM((F, D), BF16),
            pltpu.VMEM((L, D), F32), pltpu.VMEM((L, D), F32), pltpu.VMEM((L, D), BF16), pltpu.VMEM((T, 128), F32),
        ] + [scan_buf] * 8 + [
            pltpu.SemaphoreType.DMA((NC,)), pltpu.SemaphoreType.DMA((5,)),
            pltpu.SemaphoreType.DMA((NC,)), pltpu.SemaphoreType.DMA((2,)),
            pltpu.SemaphoreType.DMA((TS,)), pltpu.SemaphoreType.DMA((8,)),
        ],
        compiler_params=pltpu.CompilerParams(flags={'XLA_TPU_EVENLY_DISTRIBUTE_CRITICAL_NODES': True},
            vmem_limit_bytes=100 * 1024 * 1024),
    )(
        A_x.reshape(L, D),
        A_Lambda_re.reshape(NT, 128), A_Lambda_im.reshape(NT, 128), A_log_dt.reshape(NT, 128),
        A_Lambda_re.reshape(1, P), A_Lambda_im.reshape(1, P), A_log_dt.reshape(1, P),
        A_Dskip.reshape(1, D), B_w_r.reshape(1, D),
        A_B_re, A_B_im, A_C_re, A_C_im, B_w_gate, B_w_up, B_w_down,
    )
    return out.reshape(1, L, D)
```

```python
import jax
import jax.numpy as jnp
from jax import lax
import jax.experimental.pallas as pl
import jax.experimental.pallas.tpu as pltpu

L, D, P, F = 2048, 1024, 1024, 3584
T = 256
NC = L // T
TP = T + 4
NT = P // 128
TS = 4
AHEAD = 3
F32, BF16 = jnp.float32, jnp.bfloat16
_NT_DIMS = (((1,), (1,)), ((), ()))


def _rb(v):
    return v.astype(BF16).astype(F32)


def _row(v):
    return jnp.concatenate([v[i:i + 1] for i in range(v.shape[0])], axis=1)


def _discretize(lre, lim, ldt):
    lre, lim = lre.astype(F32), lim.astype(F32)
    dt = _rb(jnp.exp(ldt.astype(F32)))
    mag = jnp.exp(dt * lre)
    return lre, lim, mag * jnp.cos(dt * lim), mag * jnp.sin(dt * lim)


def _body(x_hbm, lre8, lim8, ldt8, dsk8, wr8,
          bre_hbm, bim_hbm, cre_hbm, cim_hbm, wg_hbm, wu_hbm, wd_hbm,
          o_hbm,
          xv, bv, cv, wg, wu, wd, buf, xnf, xnb, rs, vec,
          ur0, ui0, ur1, ui1, hr0, hi0, hr1, hi1,
          sx, sw, so, sp, st, sb):
    def xcopy(c):
        return pltpu.make_async_copy(x_hbm.at[pl.ds(c * T, T)], xv.at[pl.ds(c * T, T)], sx.at[c])

    def ocopy(c):
        return pltpu.make_async_copy(buf.at[pl.ds(c * T, T)], o_hbm.at[pl.ds(c * T, T)], so.at[c])

    wcopies = [pltpu.make_async_copy(s, d, sw.at[k]) for k, (s, d) in enumerate([
        (cre_hbm, cv.at[0]), (cim_hbm, cv.at[1]),
        (wg_hbm, wg), (wu_hbm, wu), (wd_hbm, wd)])]
    def bcopy(j):
        rows = pl.ds((j % 4) * 256, 256)
        return pltpu.make_async_copy((bre_hbm, bim_hbm)[j // 4].at[rows], bv.at[j // 4, rows], sb.at[j])

    xcopy(0).start()
    bcopy(0).start()

    _, _, ar, ai = _discretize(lre8[...], lim8[...], ldt8[...])
    vec[0:1] = _row(dsk8[...].astype(F32))
    vec[1:2] = _row(wr8[...].astype(F32))
    ubufs = ((ur0, ui0), (ur1, ui1))
    hbufs = ((hr0, hi0), (hr1, hi1))

    def stage_ln(c, q):
        rows, rr = pl.ds(c * T + q * 32, 32), pl.ds(q * 32, 32)
        x = xv[rows, :].astype(F32)
        mean = jnp.mean(x, axis=-1, keepdims=True)
        xc = x - mean
        var = _rb(jnp.mean(xc * xc, axis=-1, keepdims=True))
        den = _rb(jnp.sqrt(_rb(var + 1e-5)))
        xn = _rb(_rb(x - _rb(mean)) / den)
        xnf[rows, :] = xn
        r = jnp.sum(xn * vec[1:2], axis=-1, keepdims=True)
        lane = lax.broadcasted_iota(jnp.int32, (32, 128), 1)
        rs[rr, :] = jnp.where(lane == c, r, rs[rr, :] if c else -jnp.inf)
        buf[rows, :] = x + xn + _rb(xn * vec[0:1])
        xnb[rows, :] = xn.astype(BF16)

    def stage_a(c, pre=None, mid=None):
        slot = c % 2
        xb = xnb[pl.ds(c * T, T), :]
        for k in range(2):
            for n in range(4):
                if pre is not None:
                    pre(4 * k + n)
                u = lax.dot_general(xb, bv[k, pl.ds(n * 256, 256), :], _NT_DIMS,
                                    preferred_element_type=F32)
                for s in range(2):
                    ubufs[slot][k][pl.ds((2 * n + s) * TP, T), :] = u[:, s * 128:(s + 1) * 128]
                if mid is not None:
                    mid(4 * k + n)

    def stage_s(slot, h):
        h_re, h_im = h
        (u_re, u_im), (o_re, o_im) = ubufs[slot], hbufs[slot]
        for t in range(T):
            idx = pl.ds(t, NT, stride=TP)
            v_re, v_im = u_re[idx, :], u_im[idx, :]
            n_re = (ar * h_re + (cr * v_re - ci * v_im)) + ai * h_im
            n_im = (ar * h_im - (cr * v_im + ci * v_re)) - ai * h_re
            h_re, h_im = n_re, n_im
            o_re[idx, :] = h_re
            o_im[idx, :] = h_im
        return h_re, h_im

    def stage_c(c, cols=pl.ds(0, D)):
        slot = c % 2
        rows = pl.ds(c * T, T)
        y = buf[rows, cols]
        for k in range(2):
            hb = jnp.concatenate(
                [hbufs[slot][k][pl.ds(s * TP, T), :].astype(BF16) for s in range(NT)], axis=1)
            y = y + lax.dot_general(hb, cv[k, cols, :], _NT_DIMS, preferred_element_type=F32)
        buf[rows, cols] = y

    def coef():
        lre, lim, br, bi = _discretize(lre8[...], lim8[...], ldt8[...])
        br = br - 1.0
        inv = 2.0 / (lre * lre + lim * lim)
        cr = (br * lre + bi * lim) * inv
        ci = (bi * lre - br * lim) * inv
        return cr, ci

    def route():
        r = _rb(rs[...])
        row = (lax.broadcasted_iota(jnp.int32, r.shape, 0)
               + T * lax.broadcasted_iota(jnp.int32, r.shape, 1))
        m1 = jnp.max(r)
        i1 = jnp.min(jnp.where(r == m1, row, L))
        r2 = jnp.where(row == i1, -jnp.inf, r)
        m2 = jnp.max(r2)
        i2 = jnp.min(jnp.where(r2 == m2, row, L))
        i1 = jnp.clip(i1, 0, L - 1)
        i2 = jnp.clip(i2, 0, L - 1)
        sub = lax.broadcasted_iota(jnp.int32, (16, D), 0)
        xs = jnp.where(sub == 0, xnf[pl.ds(i1, 1), :], jnp.where(sub == 1, xnf[pl.ds(i2, 1), :], 0.0))
        return i1, i2, m1, m2, xs.astype(BF16)

    def ffn(m1, m2, xs):
        g = _rb(jnp.dot(xs, wg[...], preferred_element_type=F32))
        u = _rb(jnp.dot(xs, wu[...], preferred_element_type=F32))
        a = (_rb(g * jax.nn.sigmoid(g)) * u).astype(BF16)
        y = _rb(jnp.dot(a, wd[...], preferred_element_type=F32))
        sub1 = lax.broadcasted_iota(jnp.int32, (16, 1), 0)
        gate = _rb(jax.nn.sigmoid(jnp.where(sub1 == 0, m1, m2)))
        y = _rb(y * gate)
        return y

    cr, ci = coef()
    zero = jnp.zeros((NT, 128), F32)
    xcopy(0).wait()
    for j in range(1, AHEAD):
        bcopy(j).start()
    for q in range(8):
        stage_ln(0, q)

    def pre0(j):
        bcopy(j).wait()
        if j + AHEAD < 8:
            bcopy(j + AHEAD).start()
        if j == 1:
            xcopy(1).start()
        if j == 4:
            xcopy(1).wait()
        if j == 8 - AHEAD:
            xcopy(2).start()
            wcopies[0].start()
            wcopies[1].start()

    def mid0(j):
        if j >= 4:
            stage_ln(1, 2 * j - 8)
            stage_ln(1, 2 * j - 7)

    stage_a(0, pre=pre0, mid=mid0)
    h = (zero, zero)
    for c in range(1, NC):
        if c == 1:
            xcopy(2).wait()
            xcopy(3).start()
        if c == 2:
            wcopies[0].wait()
            wcopies[1].wait()
            xcopy(3).wait()
            for cc in range(4, NC):
                xcopy(cc).start()
            for k in range(2, 5):
                wcopies[k].start()
        if 3 <= c < NC - 1:
            xcopy(c + 1).wait()
        if c == NC - 1:
            ocopy(0).wait()
        if c + 1 < NC:
            stage_a(c, mid=lambda q: stage_ln(c + 1, q))
        else:
            stage_a(c)
            i1, i2, m1, m2, xs = route()
        h = stage_s((c - 1) % 2, h)
        if c >= 2:
            stage_c(c - 2)
        if c >= 2:
            ocopy(c - 2).start()
    for k in range(2, 5):
        wcopies[k].wait()
    y = ffn(m1, m2, xs)
    h = stage_s(1, h)
    stage_c(NC - 2)
    for c in range(1, NC - 2):
        ocopy(c).wait()
    buf[pl.ds(i1, 1), :] = buf[pl.ds(i1, 1), :] + y[0:1]
    buf[pl.ds(i2, 1), :] = buf[pl.ds(i2, 1), :] + y[1:2]

    def pcopy(i, k):
        g = pl.ds(pl.multiple_of((i // 8) * 8, 8), 8)
        return pltpu.make_async_copy(buf.at[g], o_hbm.at[g], sp.at[k])

    done = (NC - 2) * T
    p1 = i1 < done
    p2 = jnp.logical_and(i2 < done, i2 // 8 != i1 // 8)
    pl.when(p1)(lambda: pcopy(i1, 0).start())
    pl.when(p2)(lambda: pcopy(i2, 1).start())
    ocopy(NC - 2).start()
    tails = []
    for q in range(TS):
        cols = pl.ds(q * (D // TS), D // TS)
        stage_c(NC - 1, cols)
        rows = pl.ds(L - T, T)
        tails.append(pltpu.make_async_copy(buf.at[rows, cols], o_hbm.at[rows, cols], st.at[q]))
        tails[-1].start()
    pl.when(p1)(lambda: pcopy(i1, 0).wait())
    pl.when(p2)(lambda: pcopy(i2, 1).wait())
    ocopy(NC - 2).wait()
    for t in tails:
        t.wait()


@jax.jit
def pallas_parallel_sum__ssm_conv_s5__moe_arch_mod__prompt_kernel(
    A_x, A_Lambda_re, A_Lambda_im, A_B_re, A_B_im, A_C_re, A_C_im, A_log_dt, A_Dskip,
    B_x, B_w_r, B_w_gate, B_w_up, B_w_down,
):
    del B_x
    hbm = pl.BlockSpec(memory_space=pl.ANY)
    vm = pl.BlockSpec(memory_space=pltpu.VMEM)
    scan_buf = pltpu.VMEM((NT * TP, 128), F32)
    out = pl.pallas_call(
        _body,
        out_shape=jax.ShapeDtypeStruct((L, D), F32),
        in_specs=[hbm] + [vm] * 5 + [hbm] * 7,
        out_specs=hbm,
        scratch_shapes=[
            pltpu.VMEM((L, D), BF16), pltpu.VMEM((2, P, D), BF16), pltpu.VMEM((2, D, P), BF16),
            pltpu.VMEM((D, F), BF16), pltpu.VMEM((D, F), BF16), pltpu.VMEM((F, D), BF16),
            pltpu.VMEM((L, D), F32), pltpu.VMEM((L, D), F32), pltpu.VMEM((L, D), BF16), pltpu.VMEM((T, 128), F32), pltpu.VMEM((8, D), F32),
        ] + [scan_buf] * 8 + [
            pltpu.SemaphoreType.DMA((NC,)), pltpu.SemaphoreType.DMA((5,)),
            pltpu.SemaphoreType.DMA((NC,)), pltpu.SemaphoreType.DMA((2,)),
            pltpu.SemaphoreType.DMA((TS,)), pltpu.SemaphoreType.DMA((8,)),
        ],
        compiler_params=pltpu.CompilerParams(flags={'XLA_TPU_EVENLY_DISTRIBUTE_CRITICAL_NODES': True},
            vmem_limit_bytes=100 * 1024 * 1024),
    )(
        A_x.reshape(L, D),
        A_Lambda_re.reshape(NT, 128), A_Lambda_im.reshape(NT, 128), A_log_dt.reshape(NT, 128),
        A_Dskip.reshape(NT, 128), B_w_r.reshape(NT, 128),
        A_B_re, A_B_im, A_C_re, A_C_im, B_w_gate, B_w_up, B_w_down,
    )
    return out.reshape(1, L, D)
```
